```python
import os as _os
_os.environ.setdefault("JAX_PLATFORMS", "cpu")
import jax
import jax.numpy as jnp

def _softmax(x, axis=-1):
    return jax.nn.softmax(x, axis=axis)
def _gelu(x):
    return jax.nn.gelu(x, approximate=True)
def _silu(x):
    return jax.nn.silu(x)
def _sigmoid(x):
    return jax.nn.sigmoid(x)
def _layernorm(x, axis=-1, eps=1e-5):
    m = jnp.mean(x, axis=axis, keepdims=True)
    v = jnp.var(x, axis=axis, keepdims=True)
    return (x - m) / jnp.sqrt(v + eps)
def _scatter_add(tgt, idx, src, axis=0):
    return tgt.at[idx].add(src)
def _segment_sum(src, seg, n):
    return jax.ops.segment_sum(src, seg, n)
class _Rng:
    def __init__(self, key):
        self._k = key
    def _next(self):
        self._k, sub = jax.random.split(self._k)
        return sub
    def normal(self, shape):
        return jax.random.normal(self._next(), shape, dtype=jnp.bfloat16)
    def randint(self, lo, hi, shape):
        return jax.random.randint(self._next(), shape, lo, hi, dtype=jnp.int32)
    def uniform(self, shape, lo=0.0, hi=1.0):
        return jax.random.uniform(self._next(), shape, jnp.bfloat16, lo, hi)
    def permutation(self, n):
        return jax.random.permutation(self._next(), n)


kernel_name = 'sequential_preLN__sliding_local_dilated__dense_activation_relu__prompt'

def setup_inputs():
    _rng = _Rng(jax.random.key(int.from_bytes(__import__("os").urandom(4), "little")))
    _w = (lambda a: (lambda t: t.astype(jnp.bfloat16) if jnp.issubdtype(t.dtype, jnp.floating) else t)(jnp.asarray(a)))
    def _A_setup():
        B, S, D = 1, 2048, 1024
        return {
            "x": _w((lambda *s: _rng.normal(s) * 0.05)(B, S, D)),
            "wqkv": _w((lambda *s: _rng.normal(s) * 0.05)(D, 3 * D)),
            "wo": _w((lambda *s: _rng.normal(s) * 0.05)(D, D)),
        }
    _A_in = _A_setup()

    def _B_setup():
        B, S, D, Dff = 1, 2048, 1024, 3584
        return {
            "x": _w((lambda *s: _rng.normal(s) * 0.05)(B, S, D)),
            "w1": _w((lambda *s: _rng.normal(s) * 0.05)(D, Dff)),
            "w2": _w((lambda *s: _rng.normal(s) * 0.05)(Dff, D)),
        }
    _B_in = _B_setup()

    return {
        "A_x": _A_in["x"],
        "A_wqkv": _A_in["wqkv"],
        "A_wo": _A_in["wo"],
        "B_x": _B_in["x"],
        "B_w1": _B_in["w1"],
        "B_w2": _B_in["w2"],
    }

def reference(A_x, A_wqkv, A_wo, B_x, B_w1, B_w2):
    def _A_ref(x, wqkv, wo):
        B, S, D = x.shape
        H = 32; Dh = D // H
        W, dil = 8, 2
        qkv = (lambda x, *d: x.transpose(*d))((x @ wqkv).reshape(B, S, 3, H, Dh), 2, 0, 3, 1, 4)
        q, k, v = qkv[0], qkv[1], qkv[2]
        scale = Dh ** -0.5
        pos = jnp.arange(S)
        off = jnp.arange(W) * dil
        idx = pos[:, None] - off[None, :]
        mask = idx >= 0
        idx_c = jnp.where(mask, idx, 0).reshape(-1)
        kg = k[:, :, idx_c, :].reshape(B, H, S, W, Dh)
        vg = v[:, :, idx_c, :].reshape(B, H, S, W, Dh)
        logits = jnp.einsum("bhsd,bhswd->bhsw", q, kg) * scale
        logits = jnp.where(mask[None, None, :, :], logits, -1e9)
        attn = _softmax(logits, axis=-1)
        o = jnp.einsum("bhsw,bhswd->bhsd", attn, vg)
        return (lambda x, *d: x.transpose(*d))(o, 0, 2, 1, 3).reshape(B, S, D) @ wo

    def _B_ref(x, w1, w2):
        h = jnp.einsum("bsd,df->bsf", x, w1)
        zero = jnp.zeros_like(h)
        h = jnp.maximum(h, zero)
        return jnp.einsum("bsf,fd->bsd", h, w2)

    x = A_x
    h = x + _A_ref(_layernorm(x, axis=-1), A_wqkv, A_wo)
    h2 = h + _B_ref(_layernorm(h, axis=-1), B_w1, B_w2)
    return h2
```

```python
import contextlib
import functools, math
import jax, jax.numpy as jnp
from jax import lax
from jax.experimental import pallas as pl
from jax.experimental.pallas import tpu as pltpu
S, D, DFF, H, DH, W, DIL = 2048, 1024, 3584, 32, 32, 8, 2
HALO = 16
NC = D // 128
FC = 512
NF = DFF // FC
f32, bf16, i32, u32 = jnp.float32, jnp.bfloat16, jnp.int32, jnp.uint32
QS = (DH ** -0.5) * math.log2(math.e)
NT_DIMS = (((1,), (1,)), ((), ()))
FLAG = {"XLA_TPU_EVENLY_DISTRIBUTE_CRITICAL_NODES": True}

def _ln(x):
    m = jnp.mean(x, axis=-1, keepdims=True)
    xc = x - m
    v = jnp.mean(xc * xc, axis=-1, keepdims=True)
    return xc * lax.rsqrt(v + 1e-5)

def attn_b(a_s, o_s, pos0, r0, R, masked, x1="roll"):
    lane = lax.broadcasted_iota(i32, (R, 128), 1)
    odd = (lane & 1) == 1
    qs = [a_s[c, pl.ds(HALO + r0, R), :] * QS for c in range(NC)]
    lg = []
    for w in range(W):
        p = [qs[c] * a_s[NC + c, pl.ds(HALO + r0 - DIL * w, R), :] for c in range(NC)]
        while len(p) > 1:
            p = [p[i] + p[i + 1] for i in range(0, len(p), 2)]
        r3 = p[0]
        r3 = r3 + pltpu.roll(r3, 64, 1)
        if x1 == "perm":
            r3 = r3 + jnp.take_along_axis(r3, lane ^ 1, axis=1, mode="promise_in_bounds")
        else:
            r3 = r3 + jnp.where(odd, pltpu.roll(r3, 1, 1), pltpu.roll(r3, 127, 1))
        if w > 0 and masked:
            row = lax.broadcasted_iota(i32, (R, 128), 0) + (pos0 + r0)
            r3 = jnp.where(row >= DIL * w, r3, -1e9)
        lg.append(r3)
    m = functools.reduce(jnp.maximum, lg)
    es = [jnp.exp2(l - m) for l in lg]
    den = functools.reduce(jnp.add, es)
    inv = 1.0 / den
    aw = [e * inv for e in es]
    for c in range(NC):
        acc = None
        for w in range(W):
            term = aw[w] * a_s[2 * NC + c, pl.ds(HALO + r0 - DIL * w, R), :]
            acc = term if acc is None else acc + term
        o_s[c, pl.ds(r0, R), :] = acc.astype(bf16)

def make(T=256, R=8, RP=32, flags=FLAG, x1="roll", only=None, ncw2=128, bar=True, nochk=False, scopes=False, PP=4, i_perm_wo=True):
    NT = S // T
    attn = functools.partial(attn_b, x1=x1)
    NQ = 3 * NC
    def scope(n):
        return jax.named_scope(n) if scopes else contextlib.nullcontext()
    def kernel(x_hbm, wqkv_hbm, wo_hbm, w1_hbm, w2_hbm, o_ref,
               x_s, wr_s, st_s, wt_s, wor_s, wo_s, w1_s, w2_s, a_s, o_s, h_s, ln1_s, ln2_s, h1_s,
               sem_x, sem_q, sem_o, sem_1, sem_2):
        s = pl.program_id(0)
        def x_copy(t, slot):
            return pltpu.make_async_copy(x_hbm.at[pl.ds(t * T, T), :], x_s.at[slot], sem_x.at[slot])
        def q_copy(m, a):
            return pltpu.make_async_copy(wqkv_hbm.at[pl.ds(a * 128, 128), pl.ds(m * D, D)], wr_s.at[m * NC + a], sem_q.at[m * NC + a])
        def o_copy(j):
            return pltpu.make_async_copy(wo_hbm.at[:, pl.ds(j * 128, 128)], wor_s.at[j], sem_o.at[j])
        def w1_copy(j):
            return pltpu.make_async_copy(w1_hbm.at[:, pl.ds(j * FC, FC)], w1_s.at[j], sem_1.at[j])
        def w2_copy(j):
            return pltpu.make_async_copy(w2_hbm.at[pl.ds(j * FC, FC), :], w2_s.at[pl.ds(j * FC, FC), :], sem_2.at[j])

        def perm_panel(m, a, t=0):
            tr = wr_s[m * NC + a].T
            st_s[t] = pltpu.bitcast(tr, u32)
            for dp in range(16):
                g = st_s[t, pl.ds(dp, 32, stride=16), :]
                wt_s[a, pl.ds(pl.multiple_of(m * D + dp * 64, 64), 64), :] = pltpu.bitcast(g, bf16)
        def perm_wo(j):
            wu = wor_s.at[j].bitcast(u32)
            for dp in range(16):
                g = wu[pl.ds(dp, 32, stride=16), :]
                wo_s[j, pl.ds(dp * 64, 64), :] = pltpu.bitcast(g, bf16)

        def ln1(slot):
            ln1_s[...] = _ln(x_s[slot].astype(f32)).astype(bf16)
        def qkv_chunk(j):
            r0 = j * 128 if isinstance(j, int) else pl.multiple_of(j * 128, 128)
            wt = jnp.concatenate([wt_s[a, pl.ds(r0, 128), :] for a in range(NC)], axis=1)
            a_s[j, HALO:, :] = lax.dot_general(ln1_s[...], wt, NT_DIMS, preferred_element_type=f32)
        def halo():
            for j in range(NC, NQ):
                a_s[j, 0:HALO, :] = a_s[j, T:T + HALO, :]
        def wo_stage(slot):
            o = jnp.concatenate([o_s[c] for c in range(NC)], axis=1)
            for j in range(NC):
                sl = slice(j * 128, (j + 1) * 128)
                h_s[:, sl] = x_s[slot, :, sl].astype(f32) + jnp.dot(o, wo_s[j], preferred_element_type=f32)
        def ln2():
            ln2_s[...] = _ln(h_s[...]).astype(bf16)
        def w1_phase():
            ln = ln2_s[...]
            for j in range(NF):
                h1 = jnp.dot(ln, w1_s[j], preferred_element_type=f32)
                h1_s[:, j * FC:(j + 1) * FC] = jnp.maximum(h1, 0.0).astype(bf16)
        def w2_phase():
            h1 = h1_s[...]
            for n in range(D // ncw2):
                sl = slice(n * ncw2, (n + 1) * ncw2)
                r = jnp.dot(h1, w2_s[:, sl], preferred_element_type=f32)
                o_ref[:, sl] = (h_s[:, sl] + r).astype(bf16)

        def q_copy_flat(j):
            return pltpu.make_async_copy(
                wqkv_hbm.at[pl.ds(pl.multiple_of((j % NC) * 128, 128), 128), pl.ds(pl.multiple_of((j // NC) * D, D), D)],
                wr_s.at[j], sem_q.at[j])
        def o_copy_dyn(j):
            return pltpu.make_async_copy(wo_hbm.at[:, pl.ds(pl.multiple_of(j * 128, 128), 128)], wor_s.at[j], sem_o.at[j])
        def w1_copy_dyn(j):
            return pltpu.make_async_copy(w1_hbm.at[:, pl.ds(pl.multiple_of(j * FC, FC), FC)], w1_s.at[j], sem_1.at[j])
        def w2_copy_dyn(j):
            r = pl.ds(pl.multiple_of(j * FC, FC), FC)
            return pltpu.make_async_copy(w2_hbm.at[r, :], w2_s.at[r, :], sem_2.at[j])
        def prologue():
            x_copy(0, 0).start()
            @pl.loop(0, NQ)
            def _(j):
                q_copy_flat(j).start()
            x_copy(1, 1).start()
            @pl.loop(0, NC)
            def _(j):
                o_copy_dyn(j).start()
            @pl.loop(0, NF)
            def _(j):
                w1_copy_dyn(j).start()
            @pl.loop(0, NF)
            def _(j):
                w2_copy_dyn(j).start()
            for j in range(NC, NQ):
                a_s[j, 0:HALO, :] = jnp.zeros((HALO, 128), f32)
            with scope("x0ln"):
                x_copy(0, 0).wait()
                ln1(0)
            @pl.loop(0, 3)
            def _(m):
                with scope("perm"):
                    @pl.loop(0, NC // PP)
                    def _(ai):
                        for t in range(PP):
                            q_copy(m, ai * PP + t).wait()
                        for t in range(PP):
                            perm_panel(m, ai * PP + t, t)
                with scope("qkv0"):
                    @pl.loop(0, NC // 2)
                    def _(c2):
                        qkv_chunk(m * NC + c2 * 2)
                        qkv_chunk(m * NC + c2 * 2 + 1)
            with scope("attn0"):
                @pl.loop(0, T // RP)
                def _(i):
                    attn(a_s, o_s, 0, pl.multiple_of(i * RP, RP), RP, True)
                    if i_perm_wo:
                        for t in range(NC * RP // T):
                            j = i * (NC * RP // T) + t
                            o_copy(j).wait()
                            perm_wo(j)
            halo()
            if not i_perm_wo:
                with scope("permwo"):
                    @pl.loop(0, NC)
                    def _(j):
                        o_copy(j).wait()
                        perm_wo(j)
            with scope("wo0"):
                x_copy(1, 1).wait()
                wo_stage(0)
                ln1(1)
        if only is None:
            pl.when(s == 0)(prologue)

        @pl.when(s == 1)
        def _():
            for j in range(NF):
                w1_copy(j).wait()
            if not bar:
                for j in range(NF):
                    w2_copy(j).wait()
        @pl.when(s + 2 < NT)
        def _():
            x_copy(s + 2, (s + 2) % 3).start()
        @pl.when((s >= 1) & (s + 1 < NT))
        def _():
            x_copy(s + 1, (s + 1) % 3).wait()

        def block1():
          with scope("block1"):
            _block1()
        def _block1():
            for r0 in range(0, T, R):
                attn(a_s, o_s, s * T, r0, R, False)
            halo()
            w1_phase()
            if bar:
                @pl.when(s == 1)
                def _():
                    for j in range(NF):
                        w2_copy(j).wait()
            w2_phase()
            ln1(jnp.minimum(s + 1, NT - 1) % 3)
            wo_stage(s % 3)
        if only in (None, "b1"):
            pl.when((s >= 1) & (s < NT))(block1)

        def block2():
          with scope("block2"):
            _block2()
        def _block2():
            for j in range(NQ):
                qkv_chunk(j)
            ln2()
        if only in (None, "b2"):
            pl.when(s < NT - 1)(block2)

        def epilogue():
          with scope("epi"):
            _epilogue()
        def _epilogue():
            ln2()
            @pl.loop(0, NF)
            def _(j):
                h1 = jnp.dot(ln2_s[...], w1_s[j], preferred_element_type=f32)
                h1 = jnp.maximum(h1, 0.0).astype(bf16)
                h_s[...] += jnp.dot(h1, w2_s[pl.ds(pl.multiple_of(j * FC, FC), FC), :], preferred_element_type=f32)
            o_ref[...] = h_s[...].astype(bf16)
        if only is None:
            pl.when(s == NT)(epilogue)

    def fn(A_x, A_wqkv, A_wo, B_x, B_w1, B_w2):
        x = A_x.reshape(S, D)
        any_ = pl.BlockSpec(memory_space=pl.ANY)
        out = pl.pallas_call(
            kernel, grid=(NT + 1,),
            in_specs=[any_] * 5,
            out_specs=pl.BlockSpec((T, D), lambda i: (jnp.maximum(i - 1, 0), 0)),
            out_shape=jax.ShapeDtypeStruct((S, D), bf16),
            scratch_shapes=[
                pltpu.VMEM((3, T, D), bf16),
                pltpu.VMEM((NQ, 128, D), bf16),
                pltpu.VMEM((PP, 512, 128), u32),
                pltpu.VMEM((NC, 3 * D, 128), bf16),
                pltpu.VMEM((NC, D, 128), bf16),
                pltpu.VMEM((NC, D, 128), bf16),
                pltpu.VMEM((NF, D, FC), bf16),
                pltpu.VMEM((DFF, D), bf16),
                pltpu.VMEM((NQ, HALO + T, 128), f32),
                pltpu.VMEM((NC, T, 128), bf16),
                pltpu.VMEM((T, D), f32),
                pltpu.VMEM((T, D), bf16),
                pltpu.VMEM((T, D), bf16),
                pltpu.VMEM((T, DFF), bf16),
                pltpu.SemaphoreType.DMA((3,)), pltpu.SemaphoreType.DMA((NQ,)), pltpu.SemaphoreType.DMA((NC,)),
                pltpu.SemaphoreType.DMA((NF,)), pltpu.SemaphoreType.DMA((NF,)),
            ],
            compiler_params=pltpu.CompilerParams(dimension_semantics=("arbitrary",), vmem_limit_bytes=100 * 1024 * 1024, flags=flags,
                                                 disable_semaphore_checks=nochk, disable_bounds_checks=nochk),
            name="kmain",
        )(x, A_wqkv, A_wo, B_w1, B_w2)
        return out.reshape(1, S, D)
    return fn


_impl = make()


@jax.jit
def pallas_sequential_preLN__sliding_local_dilated__dense_activation_relu__prompt_kernel(
    A_x: jax.Array,
    A_wqkv: jax.Array,
    A_wo: jax.Array,
    B_x: jax.Array,
    B_w1: jax.Array,
    B_w2: jax.Array,
):
    return _impl(A_x, A_wqkv, A_wo, B_x, B_w1, B_w2)
```

```python
import math

import jax
import jax.numpy as jnp
from jax import lax
from jax.experimental import pallas as pl
from jax.experimental.pallas import tpu as pltpu

S, D, DFF = 2048, 1024, 3584
H, W, DIL = 32, 8, 2
DH = D // H
T = 256
NT = S // T
HALO = 16
NC = D // 128
NQ = 3 * NC
FC = 512
PAD = 17
QSCALE = DH ** -0.5 * math.log2(math.e)
NT_DIMS = (((1,), (1,)), ((), ()))

f32, bf16, i32, u32 = jnp.float32, jnp.bfloat16, jnp.int32, jnp.uint32


def _unpack(u):
    return pltpu.bitcast(u, bf16)


def _pack(x):
    return pltpu.bitcast(x.astype(bf16), u32)


def _layernorm(x):
    m = jnp.mean(x, axis=-1, keepdims=True)
    xc = x - m
    v = jnp.mean(xc * xc, axis=-1, keepdims=True)
    return xc * lax.rsqrt(v + 1e-5)


def _attention(a, o_s, r0, rows, pos0=None):
    odd = (lax.broadcasted_iota(i32, (rows, 128), 1) & 1) == 1
    qs = [a[c, pl.ds(HALO + r0, rows), :] * QSCALE for c in range(NC)]
    logits = []
    for w in range(W):
        p = [qs[c] * a[NC + c, pl.ds(HALO + r0 - DIL * w, rows), :] for c in range(NC)]
        while len(p) > 1:
            p = [p[i] + p[i + 1] for i in range(0, len(p), 2)]
        l = p[0]
        l = l + pltpu.roll(l, 64, 1)
        l = l + jnp.where(odd, pltpu.roll(l, 1, 1), pltpu.roll(l, 127, 1))
        if w > 0 and pos0 is not None:
            pos = lax.broadcasted_iota(i32, (rows, 128), 0) + (pos0 + r0)
            l = jnp.where(pos >= DIL * w, l, -1e9)
        logits.append(l)
    m = logits[0]
    for l in logits[1:]:
        m = jnp.maximum(m, l)
    es = [jnp.exp2(l - m) for l in logits]
    den = es[0]
    for e in es[1:]:
        den = den + e
    inv = 1.0 / den
    probs = [e * inv for e in es]
    for c in range(NC):
        acc = None
        for w in range(W):
            term = probs[w] * a[2 * NC + c, pl.ds(HALO + r0 - DIL * w, rows), :]
            acc = term if acc is None else acc + term
        o_s[c, pl.ds(r0 // 2, rows // 2), :] = _pack(acc)


def _kernel(x_hbm, wqkv_hbm, wo_hbm, w1_hbm, w2_hbm, o_ref,
            x_s, wr_s, st_s, sw_s, wtq_s, wtk_s, wtv_s, wor_s, wo_s, w1_s, w2_s,
            a0_s, a_s, o_s, h_s, ln0_s, ln1_s, ln2_s, h1_s,
            sem_x, sem_q, sem_o, sem_f):
    s = pl.program_id(0)
    wts = (wtq_s, wtk_s, wtv_s)

    def x_copy(t):
        return pltpu.make_async_copy(
            x_hbm.at[pl.ds(pl.multiple_of(t * T, T), T), :], x_s.at[t % 4], sem_x.at[t % 4])

    def q_copy(j):
        return pltpu.make_async_copy(
            wqkv_hbm.at[pl.ds(pl.multiple_of((j % NC) * 128, 128), 128),
                        pl.ds(pl.multiple_of((j // NC) * D, D), D)],
            wr_s.at[j], sem_q.at[j])

    def o_copy(j):
        return pltpu.make_async_copy(
            wo_hbm.at[:, pl.ds(pl.multiple_of(j * 128, 128), 128)], wor_s.at[j], sem_o.at[j])

    w1_copy = pltpu.make_async_copy(w1_hbm, w1_s, sem_f.at[0])
    w2_copy = pltpu.make_async_copy(w2_hbm, w2_s, sem_f.at[1])

    def regroup(stage, words, dst):
        for h in range(H):
            stage[pl.ds(h * PAD, 16), :] = words[h * 16:(h + 1) * 16]
        for dp in range(16):
            dst[pl.ds(dp * 32, 32), :] = stage[pl.ds(dp, 32, stride=PAD), :]

    def perm_panel(m, a, slot):
        regroup(st_s.at[slot], pltpu.bitcast(wr_s[m * NC + a].T, u32), wts[m].at[a])

    def perm_wo(j):
        regroup(sw_s.at[j], pltpu.bitcast(wor_s[j], u32), wo_s.at[j])

    def ln1(t, dst):
        dst[...] = _pack(_layernorm(x_s[t % 4].astype(f32)))

    def qkv_chunk(dst, nxt, m, c, src):
        r0 = c * 64 if isinstance(c, int) else pl.multiple_of(c * 64, 64)
        wt = _unpack(jnp.concatenate([wts[m][a, pl.ds(r0, 64), :] for a in range(NC)], axis=1))
        r = lax.dot_general(_unpack(src[...]), wt, NT_DIMS, preferred_element_type=f32)
        dst[m * NC + c, HALO:, :] = r
        if m > 0:
            nxt[m * NC + c, 0:HALO, :] = r[T - HALO:, :]

    def out_proj(t):
        o = _unpack(jnp.concatenate([o_s[c] for c in range(NC)], axis=1))
        for j in range(NC):
            sl = slice(j * 128, (j + 1) * 128)
            h_s[:, sl] = x_s[t % 4, :, sl].astype(f32) + jnp.dot(
                o, _unpack(wo_s[j]), preferred_element_type=f32)

    def ln2():
        ln2_s[...] = _pack(_layernorm(h_s[...]))

    def ffn():
        ln = _unpack(ln2_s[...])
        for j in range(DFF // FC):
            sl = slice(j * FC, (j + 1) * FC)
            h1 = jnp.dot(ln, w1_s[:, sl], preferred_element_type=f32)
            h1_s[:, sl] = _pack(jnp.maximum(h1, 0.0))
        h1 = _unpack(h1_s[...])
        for n in range(NC):
            sl = slice(n * 128, (n + 1) * 128)
            r = jnp.dot(h1, w2_s[:, sl], preferred_element_type=f32)
            o_ref[:, sl] = (h_s[:, sl] + r).astype(bf16)

    @pl.when(s == 0)
    def _prologue():
        x_copy(0).start()

        @pl.loop(0, NQ)
        def _(j):
            q_copy(j).start()
        x_copy(1).start()

        @pl.loop(0, NC)
        def _(j):
            o_copy(j).start()
        x_copy(2).start()

        @pl.loop(0, 1)
        def _(j):
            w1_copy.start()

        @pl.loop(0, 1)
        def _(j):
            w2_copy.start()
        for j in range(NC, NQ):
            a0_s[j, 0:HALO, :] = jnp.zeros((HALO, 128), f32)
        x_copy(0).wait()
        ln1(0, ln0_s)

        @pl.loop(0, NC // 2)
        def _(i):
            for t in range(2):
                q_copy(i * 2 + t).wait()
            for t in range(2):
                perm_panel(0, i * 2 + t, t)

        for m, n in ((0, 2), (1, 4)):
            @pl.loop(0, NC // n)
            def _(i, m=m, n=n):
                for t in range(n):
                    q_copy((m + 1) * NC + i * n + t).wait()
                for t in range(n):
                    perm_panel(m + 1, i * n + t, t)
                for t in range(n):
                    qkv_chunk(a0_s, a_s.at[1], m, i * n + t, ln0_s)

        x_copy(1).wait()
        ln1(1, ln1_s)
        for c in range(NC - 1):
            qkv_chunk(a0_s, a_s.at[1], 2, c, ln0_s)
        for j in range(NC):
            o_copy(j).wait()
        qkv_chunk(a0_s, a_s.at[1], 2, NC - 1, ln0_s)
        for j in range(NC):
            perm_wo(j)

        for r0 in range(0, T, 32):
            _attention(a0_s, o_s, r0, 32, 0 if r0 < HALO else None)
        for c in range(NC):
            for m in range(3):
                qkv_chunk(a_s.at[1], a_s.at[2], m, c, ln1_s)
        x_copy(2).wait()

    @pl.when(s == 1)
    def _():
        w1_copy.wait()
        w2_copy.wait()

    @pl.when((s >= 1) & (s + 2 < NT))
    def _():
        x_copy(s + 2).wait()

    @pl.when(s + 3 < NT)
    def _():
        x_copy(s + 3).start()

    @pl.when(s >= 1)
    def _k1():
        a = a_s.at[s % 3]
        for r0 in range(0, T, 16):
            _attention(a, o_s, r0, 16)
        ffn()

    @pl.when(s < NT - 2)
    def _k3():
        out_proj(s)
        ln1(s + 2, ln1_s)

    @pl.when(s < NT - 2)
    def _k2():
        for m in range(3):
            for c in range(NC):
                qkv_chunk(a_s.at[(s + 2) % 3], a_s.at[s % 3], m, c, ln1_s)
        ln2()

    @pl.when((s == NT - 2) | (s == NT - 1))
    def _k3_tail():
        out_proj(s)
        ln2()


@jax.jit
def pallas_sequential_preLN__sliding_local_dilated__dense_activation_relu__prompt_kernel(
    A_x: jax.Array,
    A_wqkv: jax.Array,
    A_wo: jax.Array,
    B_x: jax.Array,
    B_w1: jax.Array,
    B_w2: jax.Array,
):
    del B_x
    hbm = pl.BlockSpec(memory_space=pl.ANY)
    out = pl.pallas_call(
        _kernel,
        grid=(NT + 1,),
        in_specs=[hbm] * 5,
        out_specs=pl.BlockSpec((T, D), lambda i: (jnp.maximum(i - 1, 0), 0)),
        out_shape=jax.ShapeDtypeStruct((S, D), bf16),
        scratch_shapes=[
            pltpu.VMEM((4, T, D), bf16),
            pltpu.VMEM((NQ, 128, D), bf16),
            pltpu.VMEM((4, H * PAD, 128), u32),
            pltpu.VMEM((NC, H * PAD, 128), u32),
            pltpu.VMEM((NC, D // 2, 128), u32),
            pltpu.VMEM((NC, D // 2, 128), u32),
            pltpu.VMEM((NC, D // 2, 128), u32),
            pltpu.VMEM((NC, D, 128), bf16),
            pltpu.VMEM((NC, D // 2, 128), u32),
            pltpu.VMEM((D, DFF), bf16),
            pltpu.VMEM((DFF, D), bf16),
            pltpu.VMEM((NQ, HALO + T, 128), f32),
            pltpu.VMEM((3, NQ, HALO + T, 128), f32),
            pltpu.VMEM((NC, T // 2, 128), u32),
            pltpu.VMEM((T, D), f32),
            pltpu.VMEM((T // 2, D), u32),
            pltpu.VMEM((T // 2, D), u32),
            pltpu.VMEM((T // 2, D), u32),
            pltpu.VMEM((T // 2, DFF), u32),
            pltpu.SemaphoreType.DMA((4,)),
            pltpu.SemaphoreType.DMA((NQ,)),
            pltpu.SemaphoreType.DMA((NC,)),
            pltpu.SemaphoreType.DMA((2,)),
        ],
        compiler_params=pltpu.CompilerParams(
            dimension_semantics=("arbitrary",),
            vmem_limit_bytes=110 * 1024 * 1024,
            disable_bounds_checks=True,
            disable_semaphore_checks=True,
            flags={"XLA_TPU_EVENLY_DISTRIBUTE_CRITICAL_NODES": True},
        ),
        name="kmain",
    )(A_x.reshape(S, D), A_wqkv, A_wo, B_w1, B_w2)
    return out.reshape(1, S, D)
```
